```python
import os as _os
_os.environ.setdefault("JAX_PLATFORMS", "cpu")
import jax
import jax.numpy as jnp

def _softmax(x, axis=-1):
    return jax.nn.softmax(x, axis=axis)
def _gelu(x):
    return jax.nn.gelu(x, approximate=True)
def _silu(x):
    return jax.nn.silu(x)
def _sigmoid(x):
    return jax.nn.sigmoid(x)
def _layernorm(x, axis=-1, eps=1e-5):
    m = jnp.mean(x, axis=axis, keepdims=True)
    v = jnp.var(x, axis=axis, keepdims=True)
    return (x - m) / jnp.sqrt(v + eps)
def _scatter_add(tgt, idx, src, axis=0):
    return tgt.at[idx].add(src)
def _segment_sum(src, seg, n):
    return jax.ops.segment_sum(src, seg, n)
class _Rng:
    def __init__(self, key):
        self._k = key
    def _next(self):
        self._k, sub = jax.random.split(self._k)
        return sub
    def normal(self, shape):
        return jax.random.normal(self._next(), shape, dtype=jnp.bfloat16)
    def randint(self, lo, hi, shape):
        return jax.random.randint(self._next(), shape, lo, hi, dtype=jnp.int32)
    def uniform(self, shape, lo=0.0, hi=1.0):
        return jax.random.uniform(self._next(), shape, jnp.bfloat16, lo, hi)
    def permutation(self, n):
        return jax.random.permutation(self._next(), n)


kernel_name = 'interleave_layers__mha_block__dense_activation_mish__prompt'

def setup_inputs():
    _rng = _Rng(jax.random.key(int.from_bytes(__import__("os").urandom(4), "little")))
    _w = (lambda a: (lambda t: t.astype(jnp.bfloat16) if jnp.issubdtype(t.dtype, jnp.floating) else t)(jnp.asarray(a)))
    def _A_setup():
        B, S, D, H = 1, 2048, 512, 32
        return {
            "x": _w((lambda *s: _rng.normal(s) * 0.05)(B, S, D)),
            "wqkv": _w((lambda *s: _rng.normal(s) * 0.05)(D, 3 * D)),
            "wo": _w((lambda *s: _rng.normal(s) * 0.05)(D, D)),
        }
    _A_in = _A_setup()

    def _B_setup():
        B, S, D, F = 1, 2048, 512, 1792
        return {
            "x": _w((lambda *s: _rng.normal(s) * 0.05)(B, S, D)),
            "w1": _w((lambda *s: _rng.normal(s) * 0.4)(D, F) * (D ** -0.5)),
            "b1": _w((lambda *s: _rng.normal(s) * 0.4)(F)),
            "w2": _w((lambda *s: _rng.normal(s) * 0.4)(F, D) * (F ** -0.5)),
        }
    _B_in = _B_setup()

    return {
        "A_x": _A_in["x"],
        "A_wqkv": _A_in["wqkv"],
        "A_wo": _A_in["wo"],
        "B_x": _B_in["x"],
        "B_w1": _B_in["w1"],
        "B_b1": _B_in["b1"],
        "B_w2": _B_in["w2"],
    }

def reference(A_x, A_wqkv, A_wo, B_x, B_w1, B_b1, B_w2):
    def _A_ref(x, wqkv, wo):
        B, S, D = x.shape
        H = 32
        Dh = D // H
        qkv = (lambda x, *d: x.transpose(*d))((x @ wqkv).reshape(B, S, 3, H, Dh), 2, 0, 3, 1, 4)
        q, k, v = qkv[0], qkv[1], qkv[2]
        scores = jnp.einsum("bhqd,bhkd->bhqk", q, k) * (Dh ** -0.5)
        p = _softmax(scores, axis=-1)
        o = jnp.einsum("bhqk,bhkd->bhqd", p, v)
        return (lambda x, *d: x.transpose(*d))(o, 0, 2, 1, 3).reshape(B, S, D) @ wo

    def _B_ref(x, w1, b1, w2):
        h = jnp.einsum("bsd,df->bsf", x, w1) + b1
        sp = jnp.log1p(jnp.exp(-jnp.abs(h))) + jnp.where(h > 0, h, jnp.zeros_like(h))
        act = h * jnp.tanh(sp)
        return jnp.einsum("bsf,fd->bsd", act, w2)

    x = A_x
    x = x + _A_ref(_layernorm(x, axis=-1), A_wqkv, A_wo)
    x = x + _B_ref(_layernorm(x, axis=-1), B_w1, B_b1, B_w2)
    x = x + _A_ref(_layernorm(x, axis=-1), A_wqkv, A_wo)
    x = x + _B_ref(_layernorm(x, axis=-1), B_w1, B_b1, B_w2)
    return x
```

```python
import jax
import jax.numpy as jnp
from jax import lax
import jax.experimental.pallas as pl
import jax.experimental.pallas.tpu as pltpu

S, D, H, DH, F = 2048, 512, 32, 16, 1792
NG = D // 128
TQ = 128
CK = 128
TA = 256
TF = 512
FC = 256
NB = 4
LAG = NB - 1
QSCALE = float(DH ** -0.5 * 1.4426950408889634)


def _ln(x):
    m = jnp.mean(x, axis=-1, keepdims=True)
    d = x - m
    v = jnp.mean(d * d, axis=-1, keepdims=True)
    return d * lax.rsqrt(v + 1e-5)


def _mish(h):
    sp = jnp.log1p(jnp.exp(-jnp.abs(h))) + jnp.maximum(h, 0.0)
    return h * jnp.tanh(sp)


def _kernel(x_ref, wqkv_ref, b1_ref, wo_hbm, w1_hbm, w2_hbm, out_hbm,
            xr, ob, wo, w1, w2, kp, qp, vp, op, mref, sems, *sb):
    c_wo = pltpu.make_async_copy(wo_hbm, wo, sems.at[0])
    c_w1 = pltpu.make_async_copy(w1_hbm, w1, sems.at[1])
    c_w2 = pltpu.make_async_copy(w2_hbm, w2, sems.at[2])
    c_wo.start()
    c_w1.start()
    c_w2.start()

    def conv(t, _):
        r = pl.ds(pl.multiple_of(t * 256, 256), 256)
        xr[r, :] = x_ref[r, :].astype(jnp.float32)
        return 0

    lax.fori_loop(0, S // 256, conv, 0)

    def qkv_tile(t, _):
        r = pl.ds(pl.multiple_of(t * TA, TA), TA)
        xn = _ln(xr[r, :]).astype(jnp.bfloat16)
        q = jnp.dot(xn, wqkv_ref[:, 0:D], preferred_element_type=jnp.float32) * QSCALE
        k = jnp.dot(xn, wqkv_ref[:, D:2 * D], preferred_element_type=jnp.float32)
        v = jnp.dot(xn, wqkv_ref[:, 2 * D:3 * D], preferred_element_type=jnp.float32)
        qp[:, r] = pltpu.bitcast(q.astype(jnp.bfloat16).T, jnp.uint32)
        vp[:, r] = pltpu.bitcast(v.astype(jnp.bfloat16).T, jnp.uint32)
        kb = pltpu.bitcast(k.astype(jnp.bfloat16), jnp.uint32)
        r2 = pl.ds(pl.multiple_of(t * (TA // 2), TA // 2), TA // 2)
        for g in range(NG):
            kp[g, r2, :] = kb[:, g * 128:(g + 1) * 128]
        return 0

    class QK:
        def __init__(self, j, h):
            self.g, r = h // 8, h % 8
            self.slot = h % NB
            cols = pl.ds(pl.multiple_of(j * TQ, TQ), TQ)
            q = pltpu.bitcast(qp[h * 8:(h + 1) * 8, cols], jnp.bfloat16)
            parts = []
            if r > 0:
                parts.append(jnp.zeros((DH * r, TQ), jnp.bfloat16))
            parts.append(q)
            if r < 7:
                parts.append(jnp.zeros((DH * (7 - r), TQ), jnp.bfloat16))
            self.qpad = jnp.concatenate(parts, axis=0)
            self.m8 = None

        def chunk(self, c):
            kk = pltpu.bitcast(kp[self.g, c * (CK // 2):(c + 1) * (CK // 2), :], jnp.bfloat16)
            s = jnp.dot(kk, self.qpad, preferred_element_type=jnp.float32)
            sb[self.slot][c * CK:(c + 1) * CK, :] = s
            mc = jnp.max(s.reshape(CK // 8, 8, TQ), axis=0)
            self.m8 = mc if self.m8 is None else jnp.maximum(self.m8, mc)

        def fin(self):
            m = jnp.max(self.m8, axis=0, keepdims=True)
            mref[self.slot * 8:(self.slot + 1) * 8, :] = jnp.broadcast_to(m, (8, TQ))

    class PV:
        def __init__(self, j, h):
            self.j, self.h, self.slot = j, h, h % NB
            self.mb = mref[self.slot * 8:(self.slot + 1) * 8, :]
            self.acc = self.l8 = None

        def chunk(self, c):
            s = sb[self.slot][c * CK:(c + 1) * CK, :]
            p = jnp.exp2(s.reshape(CK // 8, 8, TQ) - self.mb[None])
            t = jnp.sum(p, axis=0)
            self.l8 = t if self.l8 is None else self.l8 + t
            w = p.reshape(CK, TQ).astype(jnp.bfloat16)
            v = pltpu.bitcast(vp[self.h * 8:(self.h + 1) * 8, c * CK:(c + 1) * CK], jnp.bfloat16)
            o = jnp.dot(v, w, preferred_element_type=jnp.float32)
            self.acc = o if self.acc is None else self.acc + o

        def fin(self):
            l = jnp.sum(self.l8, axis=0, keepdims=True)
            o = (self.acc * (1.0 / l)).astype(jnp.bfloat16)
            cols = pl.ds(pl.multiple_of(self.j * TQ, TQ), TQ)
            op[self.h * 8:(self.h + 1) * 8, cols] = pltpu.bitcast(o, jnp.uint32)

    def attn_block(j, _):
        jn = jnp.minimum(j + 1, S // TQ - 1)
        for h in range(H):
            hq = h + LAG
            q = QK(j, hq) if hq < H else QK(jn, hq - H)
            p = PV(j, h)
            for c in range(S // CK):
                q.chunk(c)
                p.chunk(c)
            p.fin()
            q.fin()
        return 0

    def attention():
        for h in range(LAG):
            q = QK(0, h)
            for c in range(S // CK):
                q.chunk(c)
            q.fin()
        lax.fori_loop(0, S // TQ, attn_block, 0)

    def ffn_tile(t, layer):
        r = pl.ds(pl.multiple_of(t * TF, TF), TF)
        ot = pltpu.bitcast(op[:, r], jnp.bfloat16)
        a = lax.dot_general(ot, wo[...], (((0,), (0,)), ((), ())),
                            preferred_element_type=jnp.float32)
        x1 = xr[r, :] + a
        xn = _ln(x1).astype(jnp.bfloat16)
        y = x1
        for f in range(F // FC):
            fs = slice(f * FC, (f + 1) * FC)
            h = jnp.dot(xn, w1[:, fs], preferred_element_type=jnp.float32)
            h = h + b1_ref[:, fs].astype(jnp.float32)
            act = _mish(h).astype(jnp.bfloat16)
            y = y + jnp.dot(act, w2[fs, :], preferred_element_type=jnp.float32)
        xr[r, :] = y
        ob[r, :] = y.astype(jnp.bfloat16)

        @pl.when(layer == 1)
        def _():
            pltpu.make_async_copy(ob.at[r, :], out_hbm.at[r, :], sems.at[3 + t]).start()

        return layer

    def layer_body(layer, _):
        lax.fori_loop(0, S // TA, qkv_tile, 0)
        attention()

        @pl.when(layer == 0)
        def _():
            c_wo.wait()
            c_w1.wait()
            c_w2.wait()

        lax.fori_loop(0, S // TF, ffn_tile, layer)
        return 0

    lax.fori_loop(0, 2, layer_body, 0)
    for t in range(S // TF):
        r = pl.ds(t * TF, TF)
        pltpu.make_async_copy(ob.at[r, :], out_hbm.at[r, :], sems.at[3 + t]).wait()


@jax.jit
def pallas_interleave_layers__mha_block__dense_activation_mish__prompt_kernel(
    A_x: jax.Array,
    A_wqkv: jax.Array,
    A_wo: jax.Array,
    B_x: jax.Array,
    B_w1: jax.Array,
    B_b1: jax.Array,
    B_w2: jax.Array,
):
    x = A_x.reshape(S, D)
    b1 = B_b1.reshape(1, F)
    anyspec = pl.BlockSpec(memory_space=pl.ANY)
    vm = pl.BlockSpec(memory_space=pltpu.VMEM)
    out = pl.pallas_call(
        _kernel,
        out_shape=jax.ShapeDtypeStruct((S, D), jnp.bfloat16),
        in_specs=[vm, vm, vm, anyspec, anyspec, anyspec],
        out_specs=anyspec,
        scratch_shapes=[
            pltpu.VMEM((S, D), jnp.float32),
            pltpu.VMEM((S, D), jnp.bfloat16),
            pltpu.VMEM((D, D), jnp.bfloat16),
            pltpu.VMEM((D, F), jnp.bfloat16),
            pltpu.VMEM((F, D), jnp.bfloat16),
            pltpu.VMEM((NG, S // 2, 128), jnp.uint32),
            pltpu.VMEM((H * 8, S), jnp.uint32),
            pltpu.VMEM((H * 8, S), jnp.uint32),
            pltpu.VMEM((H * 8, S), jnp.uint32),
            pltpu.VMEM((NB * 8, TQ), jnp.float32),
            pltpu.SemaphoreType.DMA((3 + S // TF,)),
        ] + [pltpu.VMEM((S, TQ), jnp.float32)] * NB,
        compiler_params=pltpu.CompilerParams(vmem_limit_bytes=100 * 1024 * 1024),
    )(x, A_wqkv, b1, A_wo, B_w1, B_w2)
    return out.reshape(1, S, D)
```

```python
import jax
import jax.numpy as jnp
from jax import lax
import jax.experimental.pallas as pl
import jax.experimental.pallas.tpu as pltpu

S, D, H, DH, F = 2048, 512, 32, 16, 1792
NG = D // 128
TQ = 128
CK = 128
TPB = 2
PVLAG = 16
TA = 256
TF = 256
NS = 2
FC = 128
QSCALE = float(DH ** -0.5 * 1.4426950408889634)


def _ln(x):
    m = jnp.mean(x, axis=-1, keepdims=True)
    d = x - m
    v = jnp.mean(d * d, axis=-1, keepdims=True)
    return d * lax.rsqrt(v + 1e-5)


def _mish(h):
    sp = jnp.log1p(jnp.exp(-jnp.abs(h))) + jnp.maximum(h, 0.0)
    return h * jnp.tanh(sp)


def _tree(x, op):
    vs = [x[i * 8:(i + 1) * 8] for i in range(x.shape[0] // 8)]
    while len(vs) > 1:
        vs = [op(vs[i], vs[i + 1]) for i in range(0, len(vs), 2)]
    return vs[0]


def _kernel(x_ref, wqkv_ref, b1_ref, wo_hbm, w1_hbm, w2_hbm, out_hbm,
            xr, ob, wo, w1, w2, kp, qp, vp, op, sems):
    c_wo = pltpu.make_async_copy(wo_hbm, wo, sems.at[0])
    c_w1 = pltpu.make_async_copy(w1_hbm, w1, sems.at[1])
    c_w2 = pltpu.make_async_copy(w2_hbm, w2, sems.at[2])
    c_wo.start()
    c_w1.start()
    c_w2.start()

    def conv(t, _):
        r = pl.ds(pl.multiple_of(t * 256, 256), 256)
        xr[r, :] = x_ref[r, :].astype(jnp.float32)
        return 0

    lax.fori_loop(0, S // 256, conv, 0)

    def qkv_tile(t):
        r = pl.ds(t * TA, TA)
        xn = _ln(xr[r, :]).astype(jnp.bfloat16)
        q = jnp.dot(xn, wqkv_ref[:, 0:D], preferred_element_type=jnp.float32) * QSCALE
        k = jnp.dot(xn, wqkv_ref[:, D:2 * D], preferred_element_type=jnp.float32)
        v = jnp.dot(xn, wqkv_ref[:, 2 * D:3 * D], preferred_element_type=jnp.float32)
        qp[:, r] = pltpu.bitcast(q.astype(jnp.bfloat16).T, jnp.uint32)
        vp[:, r] = pltpu.bitcast(v.astype(jnp.bfloat16).T, jnp.uint32)
        kb = pltpu.bitcast(k.astype(jnp.bfloat16), jnp.uint32)
        r2 = pl.ds(t * (TA // 2), TA // 2)
        for g in range(NG):
            kp[g, r2, :] = kb[:, g * 128:(g + 1) * 128]

    class Item:
        def __init__(self, j, h):
            self.h, self.g, r = h, h // 8, h % 8
            self.cols = pl.ds(pl.multiple_of(j * TQ, TQ), TQ)
            q = pltpu.bitcast(qp[h * 8:(h + 1) * 8, self.cols], jnp.bfloat16)
            parts = []
            if r > 0:
                parts.append(jnp.zeros((DH * r, TQ), jnp.bfloat16))
            parts.append(q)
            if r < 7:
                parts.append(jnp.zeros((DH * (7 - r), TQ), jnp.bfloat16))
            self.qpad = jnp.concatenate(parts, axis=0)
            self.acc = self.l8 = self.m = None
            self.pend = []

        def qk(self, c):
            kk = pltpu.bitcast(kp[self.g, c * (CK // 2):(c + 1) * (CK // 2), :], jnp.bfloat16)
            s = jnp.dot(kk, self.qpad, preferred_element_type=jnp.float32)
            cm = jnp.max(_tree(s, jnp.maximum), axis=0, keepdims=True)
            if self.m is None:
                self.m, alpha = cm, None
            else:
                mn = jnp.maximum(self.m, cm)
                alpha = jnp.exp2(self.m - mn)
                self.m = mn
            mb = jnp.broadcast_to(self.m, (8, TQ))
            p = jnp.exp2(s.reshape(CK // 8, 8, TQ) - mb[None]).reshape(CK, TQ)
            t = _tree(p, jnp.add)
            self.l8 = t if alpha is None else self.l8 * alpha + t
            self.pend.append((p.astype(jnp.bfloat16), alpha))

        def pv(self, c):
            w, alpha = self.pend.pop(0)
            v = pltpu.bitcast(vp[self.h * 8:(self.h + 1) * 8, c * CK:(c + 1) * CK], jnp.bfloat16)
            o = jnp.dot(v, w, preferred_element_type=jnp.float32)
            self.acc = o if self.acc is None else self.acc * alpha + o

        def fin(self):
            l = jnp.sum(self.l8, axis=0, keepdims=True)
            o = (self.acc * (1.0 / l)).astype(jnp.bfloat16)
            op[self.h * 8:(self.h + 1) * 8, self.cols] = pltpu.bitcast(o, jnp.uint32)

    def attn_block(b, _):
        nc = S // CK
        total = TPB * H * nc
        cur = {}
        for step in range(total + PVLAG):
            if step < total:
                i, c = divmod(step, nc)
                if c == 0:
                    cur[i] = Item(b * TPB + i // H, i % H)
                cur[i].qk(c)
            if step >= PVLAG:
                i, c = divmod(step - PVLAG, nc)
                cur[i].pv(c)
                if c == nc - 1:
                    cur[i].fin()
                    del cur[i]
        return 0

    def ffn_tiles(t, layer):
        rs = [pl.ds(pl.multiple_of((t * NS + i) * TF, TF), TF) for i in range(NS)]
        ys, xns = [], []
        for r in rs:
            ot = pltpu.bitcast(op[:, r], jnp.bfloat16)
            a = lax.dot_general(ot, wo[...], (((0,), (0,)), ((), ())),
                                preferred_element_type=jnp.float32)
            x1 = xr[r, :] + a
            ys.append(x1)
            xns.append(_ln(x1).astype(jnp.bfloat16))
        for i in range(NS):
            for f in range(F // FC):
                fs = slice(f * FC, (f + 1) * FC)
                h = jnp.dot(xns[i], w1[:, fs], preferred_element_type=jnp.float32)
                h = h + b1_ref[:, fs].astype(jnp.float32)
                act = _mish(h).astype(jnp.bfloat16)
                ys[i] = ys[i] + jnp.dot(act, w2[fs, :], preferred_element_type=jnp.float32)
        for i, r in enumerate(rs):
            xr[r, :] = ys[i]
            ob[r, :] = ys[i].astype(jnp.bfloat16)

        @pl.when(layer == 1)
        def _():
            rr = pl.ds(pl.multiple_of(t * NS * TF, NS * TF), NS * TF)
            pltpu.make_async_copy(ob.at[rr, :], out_hbm.at[rr, :], sems.at[3 + t]).start()

        return layer

    def layer_body(layer, _):
        for t in range(S // TA):
            qkv_tile(t)
        lax.fori_loop(0, S // TQ // TPB, attn_block, 0)

        @pl.when(layer == 0)
        def _():
            c_wo.wait()
            c_w1.wait()
            c_w2.wait()

        lax.fori_loop(0, S // TF // NS, ffn_tiles, layer)
        return 0

    lax.fori_loop(0, 2, layer_body, 0)
    for t in range(S // TF // NS):
        rr = pl.ds(t * NS * TF, NS * TF)
        pltpu.make_async_copy(ob.at[rr, :], out_hbm.at[rr, :], sems.at[3 + t]).wait()


@jax.jit
def pallas_interleave_layers__mha_block__dense_activation_mish__prompt_kernel(
    A_x: jax.Array,
    A_wqkv: jax.Array,
    A_wo: jax.Array,
    B_x: jax.Array,
    B_w1: jax.Array,
    B_b1: jax.Array,
    B_w2: jax.Array,
):
    x = A_x.reshape(S, D)
    b1 = B_b1.reshape(1, F)
    anyspec = pl.BlockSpec(memory_space=pl.ANY)
    vm = pl.BlockSpec(memory_space=pltpu.VMEM)
    out = pl.pallas_call(
        _kernel,
        out_shape=jax.ShapeDtypeStruct((S, D), jnp.bfloat16),
        in_specs=[vm, vm, vm, anyspec, anyspec, anyspec],
        out_specs=anyspec,
        scratch_shapes=[
            pltpu.VMEM((S, D), jnp.float32),
            pltpu.VMEM((S, D), jnp.bfloat16),
            pltpu.VMEM((D, D), jnp.bfloat16),
            pltpu.VMEM((D, F), jnp.bfloat16),
            pltpu.VMEM((F, D), jnp.bfloat16),
            pltpu.VMEM((NG, S // 2, 128), jnp.uint32),
            pltpu.VMEM((H * 8, S), jnp.uint32),
            pltpu.VMEM((H * 8, S), jnp.uint32),
            pltpu.VMEM((H * 8, S), jnp.uint32),
            pltpu.SemaphoreType.DMA((3 + S // TF // NS,)),
        ],
        compiler_params=pltpu.CompilerParams(vmem_limit_bytes=100 * 1024 * 1024),
    )(x, A_wqkv, b1, A_wo, B_w1, B_w2)
    return out.reshape(1, S, D)
```

```python
import jax
import jax.numpy as jnp
from jax import lax
import jax.experimental.pallas as pl
import jax.experimental.pallas.tpu as pltpu

S, D, H, DH, F = 2048, 512, 32, 16, 1792
NG = D // 128
TQ = 128
CK = 128
TPB = 2
PVLAG = 16
TA = 256
NFIRST = 2
TF = 256
NS = 2
FC = 128
NFT = S // TF // NS
QSCALE = float(DH ** -0.5 * 1.4426950408889634)


def _ln(x):
    m = jnp.mean(x, axis=-1, keepdims=True)
    d = x - m
    v = jnp.mean(d * d, axis=-1, keepdims=True)
    return d * lax.rsqrt(v + 1e-5)


def _mish(h):
    sp = jnp.log1p(jnp.exp(-jnp.abs(h))) + jnp.maximum(h, 0.0)
    return h * jnp.tanh(sp)


def _tree(x, op):
    vs = [x[i * 8:(i + 1) * 8] for i in range(x.shape[0] // 8)]
    while len(vs) > 1:
        vs = [op(vs[i], vs[i + 1]) for i in range(0, len(vs), 2)]
    return vs[0]


def _pack(x):
    return pltpu.bitcast(x, jnp.uint32)


def _unpack(x):
    return pltpu.bitcast(x, jnp.bfloat16)


def _kernel(b1_ref, x_hbm, wqkv_hbm, wo_hbm, w1_hbm, w2_hbm, out_hbm,
            xin, wqkv, xr, ob, wo, w1, w2, kp, qp, vp, op, on0, xn0, wsems, isems, osems):
    nh = NFIRST * TA
    c_wqkv = pltpu.make_async_copy(wqkv_hbm, wqkv, isems.at[0])
    c_x0 = pltpu.make_async_copy(x_hbm.at[pl.ds(0, nh), :], xin.at[pl.ds(0, nh), :], isems.at[1])
    c_x1 = pltpu.make_async_copy(x_hbm.at[pl.ds(nh, S - nh), :], xin.at[pl.ds(nh, S - nh), :],
                                 isems.at[2])
    c_wo = pltpu.make_async_copy(wo_hbm, wo, wsems.at[0])
    c_w1 = pltpu.make_async_copy(w1_hbm, w1, wsems.at[1])
    c_w2 = pltpu.make_async_copy(w2_hbm, w2, wsems.at[2])

    def conv(t, _):
        r = pl.ds(pl.multiple_of(t * TA, TA), TA)
        xr[r, :] = xin[r, :].astype(jnp.float32)
        return 0

    c_wqkv.start()
    c_x0.start()
    c_x0.wait()
    c_x1.start()
    lax.fori_loop(0, NFIRST, conv, 0)
    c_wqkv.wait()

    def qkv_tile(t, xn=None):
        r = pl.ds(t * TA, TA)
        if xn is None:
            xn = _ln(xr[r, :]).astype(jnp.bfloat16)
        q = jnp.dot(xn, wqkv[:, 0:D], preferred_element_type=jnp.float32) * QSCALE
        qp[:, r] = _pack(q.astype(jnp.bfloat16).T)
        v = jnp.dot(xn, wqkv[:, 2 * D:3 * D], preferred_element_type=jnp.float32)
        vp[:, r] = _pack(v.astype(jnp.bfloat16).T)
        k = jnp.dot(xn, wqkv[:, D:2 * D], preferred_element_type=jnp.float32)
        kb = _pack(k.astype(jnp.bfloat16))
        r2 = pl.ds(t * (TA // 2), TA // 2)
        for g in range(NG):
            kp[g, r2, :] = kb[:, g * 128:(g + 1) * 128]

    class Item:
        def __init__(self, j, h):
            self.h, self.g, r = h, h // 8, h % 8
            self.cols = pl.ds(pl.multiple_of(j * TQ, TQ), TQ)
            q = _unpack(qp[h * 8:(h + 1) * 8, self.cols])
            parts = []
            if r > 0:
                parts.append(jnp.zeros((DH * r, TQ), jnp.bfloat16))
            parts.append(q)
            if r < 7:
                parts.append(jnp.zeros((DH * (7 - r), TQ), jnp.bfloat16))
            self.qpad = jnp.concatenate(parts, axis=0)
            self.acc = self.l8 = self.m = None
            self.pend = []

        def qk(self, c):
            kk = _unpack(kp[self.g, c * (CK // 2):(c + 1) * (CK // 2), :])
            s = jnp.dot(kk, self.qpad, preferred_element_type=jnp.float32)
            cm = jnp.max(_tree(s, jnp.maximum), axis=0, keepdims=True)
            if self.m is None:
                self.m, alpha = cm, None
            else:
                mn = jnp.maximum(self.m, cm)
                alpha = jnp.exp2(self.m - mn)
                self.m = mn
            mb = jnp.broadcast_to(self.m, (8, TQ))
            p = jnp.exp2(s.reshape(CK // 8, 8, TQ) - mb[None]).reshape(CK, TQ)
            t = _tree(p, jnp.add)
            self.l8 = t if alpha is None else self.l8 * alpha + t
            self.pend.append((p.astype(jnp.bfloat16), alpha))

        def pv(self, c):
            w, alpha = self.pend.pop(0)
            v = _unpack(vp[self.h * 8:(self.h + 1) * 8, c * CK:(c + 1) * CK])
            o = jnp.dot(v, w, preferred_element_type=jnp.float32)
            self.acc = o if self.acc is None else self.acc * alpha + o

        def fin(self):
            l = jnp.sum(self.l8, axis=0, keepdims=True)
            o = (self.acc * (1.0 / l)).astype(jnp.bfloat16)
            op[self.h * 8:(self.h + 1) * 8, self.cols] = _pack(o)

    def attn_block(b, _):
        nc = S // CK
        total = TPB * H * nc
        cur = {}
        for step in range(total + PVLAG):
            if step < total:
                i, c = divmod(step, nc)
                if c == 0:
                    cur[i] = Item(b * TPB + i // H, i % H)
                cur[i].qk(c)
            if step >= PVLAG:
                i, c = divmod(step - PVLAG, nc)
                cur[i].pv(c)
                if c == nc - 1:
                    cur[i].fin()
                    del cur[i]
        return 0

    def ffn_tiles(t, layer):
        rs = [pl.ds(pl.multiple_of((t * NS + i) * TF, TF), TF) for i in range(NS)]
        ys, xns = [], []
        for i, r in enumerate(rs):
            if i == 0:
                a = jnp.dot(_unpack(on0[...]), wo[...], preferred_element_type=jnp.float32)
                tn = jnp.minimum(t + 1, NFT - 1)
                rn = pl.ds(pl.multiple_of(tn * (NS * TF), TF), TF)
                on0[...] = _pack(_unpack(op[:, rn]).T)
            else:
                a = lax.dot_general(_unpack(op[:, r]), wo[...], (((0,), (0,)), ((), ())),
                                    preferred_element_type=jnp.float32)
            x1 = xr[r, :] + a
            ys.append(x1)
            xns.append(_ln(x1).astype(jnp.bfloat16))
        for i in range(NS):
            for f in range(F // FC):
                fs = pl.ds(f * FC, FC)
                h = jnp.dot(xns[i], w1[:, fs], preferred_element_type=jnp.float32)
                h = h + b1_ref[fs].reshape(1, FC).astype(jnp.float32)
                act = _mish(h).astype(jnp.bfloat16)
                ys[i] = ys[i] + jnp.dot(act, w2[fs, :], preferred_element_type=jnp.float32)
        for i, r in enumerate(rs):
            xr[r, :] = ys[i]
            ob[r, :] = ys[i].astype(jnp.bfloat16)

        @pl.when(layer == 1)
        def _():
            rr = pl.ds(pl.multiple_of(t * (NS * TF), NS * TF), NS * TF)
            pltpu.make_async_copy(ob.at[rr, :], out_hbm.at[rr, :], osems.at[t]).start()

        return layer

    def layer_body(layer, _):
        for t in range(NFIRST - 1):
            qkv_tile(t)
        xn0[...] = _pack(_ln(xr[pl.ds((NFIRST - 1) * TA, TA), :]).astype(jnp.bfloat16))

        @pl.when(layer == 0)
        def _():
            c_x1.wait()
            c_wo.start()
            c_w1.start()
            c_w2.start()
            lax.fori_loop(NFIRST, S // TA, conv, 0)

        qkv_tile(NFIRST - 1, _unpack(xn0[...]))
        for t in range(NFIRST, S // TA):
            qkv_tile(t)

        lax.fori_loop(0, S // TQ // TPB, attn_block, 0)

        @pl.when(layer == 0)
        def _():
            c_wo.wait()
            c_w1.wait()
            c_w2.wait()

        on0[...] = _pack(_unpack(op[:, 0:TF]).T)
        lax.fori_loop(0, NFT, ffn_tiles, layer)
        return 0

    lax.fori_loop(0, 2, layer_body, 0)
    for t in range(NFT):
        rr = pl.ds(t * NS * TF, NS * TF)
        pltpu.make_async_copy(ob.at[rr, :], out_hbm.at[rr, :], osems.at[t]).wait()


@jax.jit
def pallas_interleave_layers__mha_block__dense_activation_mish__prompt_kernel(
    A_x: jax.Array,
    A_wqkv: jax.Array,
    A_wo: jax.Array,
    B_x: jax.Array,
    B_w1: jax.Array,
    B_b1: jax.Array,
    B_w2: jax.Array,
):
    x = A_x.reshape(S, D)
    anyspec = pl.BlockSpec(memory_space=pl.ANY)
    vm = pl.BlockSpec(memory_space=pltpu.VMEM)
    out = pl.pallas_call(
        _kernel,
        out_shape=jax.ShapeDtypeStruct((S, D), jnp.bfloat16),
        in_specs=[vm, anyspec, anyspec, anyspec, anyspec, anyspec],
        out_specs=anyspec,
        scratch_shapes=[
            pltpu.VMEM((S, D), jnp.bfloat16),
            pltpu.VMEM((D, 3 * D), jnp.bfloat16),
            pltpu.VMEM((S, D), jnp.float32),
            pltpu.VMEM((S, D), jnp.bfloat16),
            pltpu.VMEM((D, D), jnp.bfloat16),
            pltpu.VMEM((D, F), jnp.bfloat16),
            pltpu.VMEM((F, D), jnp.bfloat16),
            pltpu.VMEM((NG, S // 2, 128), jnp.uint32),
            pltpu.VMEM((H * 8, S), jnp.uint32),
            pltpu.VMEM((H * 8, S), jnp.uint32),
            pltpu.VMEM((H * 8, S), jnp.uint32),
            pltpu.VMEM((TF // 2, D), jnp.uint32),
            pltpu.VMEM((TA // 2, D), jnp.uint32),
            pltpu.SemaphoreType.DMA((3,)),
            pltpu.SemaphoreType.DMA((3,)),
            pltpu.SemaphoreType.DMA((NFT,)),
        ],
        compiler_params=pltpu.CompilerParams(vmem_limit_bytes=100 * 1024 * 1024),
    )(B_b1, x, A_wqkv, A_wo, B_w1, B_w2)
    return out.reshape(1, S, D)
```
